```python
import jax
import jax.numpy as jnp

def _softmax(x, axis=-1):
    return jax.nn.softmax(x, axis=axis)
def _gelu(x):
    return jax.nn.gelu(x, approximate=True)
def _silu(x):
    return jax.nn.silu(x)
def _sigmoid(x):
    return jax.nn.sigmoid(x)
def _layernorm(x, axis=-1, eps=1e-5):
    m = jnp.mean(x, axis=axis, keepdims=True)
    v = jnp.var(x, axis=axis, keepdims=True)
    return (x - m) / jnp.sqrt(v + eps)
def _scatter_add(tgt, idx, src, axis=0):
    return tgt.at[idx].add(src)
def _segment_sum(src, seg, n):
    return jax.ops.segment_sum(src, seg, n)
class _Rng:
    def __init__(self, key):
        self._k = key
    def _next(self):
        self._k, sub = jax.random.split(self._k)
        return sub
    def normal(self, shape):
        return jax.random.normal(self._next(), shape, dtype=jnp.bfloat16)
    def randint(self, lo, hi, shape):
        return jax.random.randint(self._next(), shape, lo, hi, dtype=jnp.int32)
    def uniform(self, shape, lo=0.0, hi=1.0):
        return jax.random.uniform(self._next(), shape, jnp.bfloat16, lo, hi)
    def permutation(self, n):
        return jax.random.permutation(self._next(), n)


kernel_name = 'recurrent_scan__sliding_block_cached__moe_arch_mod__prompt'

def setup_inputs():
    _rng = _Rng(jax.random.key(int.from_bytes(__import__("os").urandom(4), "little")))
    _w = (lambda a: (lambda t: t.astype(jnp.bfloat16) if jnp.issubdtype(t.dtype, jnp.floating) else t)(jnp.asarray(a)))
    def _A_setup():
        B, Sq, D = 1, 2048, 640
        Hq, Hkv, Sk, Dh = 32, 32, 2048, 192
        assert Hq % Hkv == 0, (Hq, Hkv)
        return {
            "x": _w((lambda *s: _rng.normal(s) * 0.05)(B, Sq, D)),
            "k_cache": _w((lambda *s: _rng.normal(s) * 0.05)(B, Hkv, Sk, Dh)),
            "v_cache": _w((lambda *s: _rng.normal(s) * 0.05)(B, Hkv, Sk, Dh)),
            "wq": _w((lambda *s: _rng.normal(s) * 0.05)(D, Hq * Dh) * (D ** -0.5)),
            "wo": _w((lambda *s: _rng.normal(s) * 0.05)(Hq * Dh, D) * ((Hq * Dh) ** -0.5)),
        }
    _A_in = _A_setup()

    def _B_setup():
        B, S, D, F, C = 1, 2048, 640, 1536, 2
        return {
            "x": _w((lambda *s: _rng.normal(s) * 0.05)(B, S, D)),
            "w_r": _w((lambda *s: _rng.normal(s) * 0.05)(D)),
            "w_gate": _w((lambda *s: _rng.normal(s) * 0.05)(D, F)),
            "w_up": _w((lambda *s: _rng.normal(s) * 0.05)(D, F)),
            "w_down": _w((lambda *s: _rng.normal(s) * 0.05)(F, D)),
        }
    _B_in = _B_setup()

    return {
        "A_x": _A_in["x"],
        "A_k_cache": _A_in["k_cache"],
        "A_v_cache": _A_in["v_cache"],
        "A_wq": _A_in["wq"],
        "A_wo": _A_in["wo"],
        "B_x": _B_in["x"],
        "B_w_r": _B_in["w_r"],
        "B_w_gate": _B_in["w_gate"],
        "B_w_up": _B_in["w_up"],
        "B_w_down": _B_in["w_down"],
    }

def reference(A_x, A_k_cache, A_v_cache, A_wq, A_wo, B_x, B_w_r, B_w_gate, B_w_up, B_w_down):
    def _A_ref(x, k_cache, v_cache, wq, wo):
        B, Sq, D = x.shape
        Hq, Dh = 32, 192
        Hkv, Sk = k_cache.shape[1], k_cache.shape[2]
        W = min(4096, max(256, Sk // 4))
        rep = Hq // Hkv
        q = (lambda x, *d: x.transpose(*d))((x @ wq).reshape(B, Sq, Hq, Dh), 0, 2, 1, 3)
        k = jnp.repeat(k_cache[:, :, Sk - W:, :], rep, axis=1)
        v = jnp.repeat(v_cache[:, :, Sk - W:, :], rep, axis=1)
        scores = jnp.einsum("bhqd,bhkd->bhqk", q, k) * (Dh ** -0.5)
        p = _softmax(scores, axis=-1)
        o = jnp.einsum("bhqk,bhkd->bhqd", p, v)
        return (lambda x, *d: x.transpose(*d))(o, 0, 2, 1, 3).reshape(B, Sq, Hq * Dh) @ wo

    def _B_ref(x, w_r, w_gate, w_up, w_down):
        B, S, D = x.shape
        C = 2
        r = x @ w_r
        idx = jnp.argsort(-r, axis=-1)[:, :C]
        idx_e = jnp.repeat(idx.reshape(B, C, 1), D, axis=2)
        x_sel = jnp.take_along_axis(x, idx_e, axis=1)
        g = _silu(x_sel @ w_gate)
        u = x_sel @ w_up
        y = (g * u) @ w_down
        r_sel = _sigmoid(jnp.take_along_axis(r, idx, axis=1))
        y = y * r_sel.reshape(B, C, 1)
        b_off = (jnp.arange(B) * S).reshape(B, 1)
        flat_idx = (idx + b_off).reshape(B * C)
        zero = (x * 0.0).reshape(B * S, D)
        upd = _scatter_add(zero, flat_idx, y.reshape(B * C, D), axis=0)
        return x + upd.reshape(B, S, D)

    x = A_x
    xn = _layernorm(x, axis=-1)
    s = _A_ref(xn, A_k_cache, A_v_cache, A_wq, A_wo)
    g = _silu(_B_ref(xn, B_w_r, B_w_gate, B_w_up, B_w_down))
    return x + s * g
```

```python
import functools
import jax
import jax.numpy as jnp
import numpy as np
from jax import lax
from jax.experimental import pallas as pl
from jax.experimental.pallas import tpu as pltpu

S, D, H, DH, SK, F = 2048, 640, 32, 192, 2048, 1536
W = 512
PAIR = 2 * DH
LOG2E = 1.4426950408889634


def build(TM=1024):
    def kernel(x_ref, kT_ref, vT_ref, wq_ref, wo_ref, wr_ref, wg_ref, wu_ref, wd_ref, o_ref,
               xn_ref, acc_ref, upd_ref, sel_ref):
        i = pl.program_id(0)

        @pl.when(i == 0)
        def _():
            x = x_ref[...].astype(jnp.float32)
            m = jnp.mean(x, axis=-1, keepdims=True)
            xc = x - m
            v = jnp.mean(xc * xc, axis=-1, keepdims=True)
            xn = (xc / jnp.sqrt(v + 1e-5)).astype(jnp.bfloat16)
            xn_ref[...] = xn
            xnf = xn.astype(jnp.float32)
            r = jnp.sum(xnf * wr_ref[...].astype(jnp.float32), axis=-1, keepdims=True)
            row = lax.broadcasted_iota(jnp.int32, (S, 1), 0)
            m1 = jnp.max(r, axis=0, keepdims=True)
            i1 = jnp.min(jnp.where(r == m1, row, S), axis=0, keepdims=True)
            r2 = jnp.where(row == i1, -jnp.inf, r)
            m2 = jnp.max(r2, axis=0, keepdims=True)
            i2 = jnp.min(jnp.where(r2 == m2, row, S), axis=0, keepdims=True)
            x1 = jnp.sum(jnp.where(row == i1, xnf, 0.0), axis=0, keepdims=True)
            x2 = jnp.sum(jnp.where(row == i2, xnf, 0.0), axis=0, keepdims=True)
            r8 = lax.broadcasted_iota(jnp.int32, (8, 1), 0)
            xs = jnp.where(r8 == 0, x1, jnp.where(r8 == 1, x2, 0.0)).astype(jnp.bfloat16)
            g = jnp.dot(xs, wg_ref[...], preferred_element_type=jnp.float32)
            u = jnp.dot(xs, wu_ref[...], preferred_element_type=jnp.float32)
            hdn = (g * jax.nn.sigmoid(g) * u).astype(jnp.bfloat16)
            y = jnp.dot(hdn, wd_ref[...], preferred_element_type=jnp.float32)
            rs = jax.nn.sigmoid(jnp.where(r8 == 0, m1, m2))
            upd_ref[...] = y * rs
            sel_ref[...] = jnp.where(row == i1, 1, jnp.where(row == i2, 2, 0))
            acc_ref[...] = jnp.zeros_like(acc_ref)

        z = jnp.zeros((64, W), jnp.bfloat16)
        k0 = jnp.concatenate([kT_ref[0:192, :], z], axis=0)
        k1 = jnp.concatenate([z, kT_ref[192:384, :]], axis=0)
        v0 = jnp.concatenate([vT_ref[0:192, :], z], axis=0)
        v1 = jnp.concatenate([z, vT_ref[192:384, :]], axis=0)
        c = (DH ** -0.5) * LOG2E
        NT = (((1,), (1,)), ((), ()))

        def body(j, carry):
            rows = pl.ds(pl.multiple_of(j * TM, TM), TM)
            q = (jnp.dot(xn_ref[rows, :], wq_ref[...], preferred_element_type=jnp.float32) * c).astype(jnp.bfloat16)
            os_ = []
            ls = []
            for (qq, kk, vv) in ((q[:, 0:256], k0, v0), (q[:, 128:384], k1, v1)):
                s = jnp.dot(qq, kk, preferred_element_type=jnp.float32)
                mx = jnp.max(s, axis=-1, keepdims=True)
                p = jnp.exp2(s - mx)
                l = jnp.sum(p, axis=-1, keepdims=True)
                o = lax.dot_general(p.astype(jnp.bfloat16), vv, NT, preferred_element_type=jnp.float32)
                os_.append(o * (1.0 / l))
            o2 = jnp.concatenate([os_[0][:, 0:128], os_[0][:, 128:256] + os_[1][:, 0:128], os_[1][:, 128:256]], axis=1)
            acc_ref[rows, :] += jnp.dot(o2.astype(jnp.bfloat16), wo_ref[...], preferred_element_type=jnp.float32)
            return carry

        lax.fori_loop(0, S // TM, body, 0)

        @pl.when(i == pl.num_programs(0) - 1)
        def _():
            sel = sel_ref[...]
            upd = jnp.where(sel == 1, upd_ref[0:1, :], jnp.where(sel == 2, upd_ref[1:2, :], 0.0))
            t = xn_ref[...].astype(jnp.float32) + upd
            g = t * jax.nn.sigmoid(t)
            o_ref[...] = (x_ref[...].astype(jnp.float32) + acc_ref[...] * g).astype(o_ref.dtype)

    def f(A_x, A_k_cache, A_v_cache, A_wq, A_wo, B_x, B_w_r, B_w_gate, B_w_up, B_w_down):
        x = A_x.reshape(S, D)
        kT = jnp.swapaxes(A_k_cache, 2, 3).reshape(H * DH, SK)
        vT = jnp.swapaxes(A_v_cache, 2, 3).reshape(H * DH, SK)
        wr = B_w_r.reshape(1, D)
        full = lambda shape: pl.BlockSpec(shape, lambda i: (0,) * len(shape))
        out = pl.pallas_call(
            kernel,
            grid=(H // 2,),
            in_specs=[
                full((S, D)),
                pl.BlockSpec((PAIR, W), lambda i: (i, SK // W - 1)),
                pl.BlockSpec((PAIR, W), lambda i: (i, SK // W - 1)),
                pl.BlockSpec((D, PAIR), lambda i: (0, i)),
                pl.BlockSpec((PAIR, D), lambda i: (i, 0)),
                full((1, D)), full((D, F)), full((D, F)), full((F, D)),
            ],
            out_specs=full((S, D)),
            out_shape=jax.ShapeDtypeStruct((S, D), jnp.bfloat16),
            scratch_shapes=[
                pltpu.VMEM((S, D), jnp.bfloat16),
                pltpu.VMEM((S, D), jnp.float32),
                pltpu.VMEM((8, D), jnp.float32),
                pltpu.VMEM((S, 1), jnp.int32),
            ],
            compiler_params=pltpu.CompilerParams(
                dimension_semantics=("arbitrary",), vmem_limit_bytes=100 * 1024 * 1024),
        )(x, kT, vT, A_wq, A_wo, wr, B_w_gate, B_w_up, B_w_down)
        return out.reshape(1, S, D)
    return f

pallas_recurrent_scan__sliding_block_cached__moe_arch_mod__prompt_kernel = jax.jit(build())
```

```python
import functools
import jax
import jax.numpy as jnp
import numpy as np
from jax import lax
from jax.experimental import pallas as pl
from jax.experimental.pallas import tpu as pltpu

S, D, H, DH, SK, F = 2048, 640, 32, 192, 2048, 1536
W = 512
PAIR = 2 * DH
NP = H // 2
LOG2E = 1.4426950408889634
f32 = jnp.float32
bf16 = jnp.bfloat16
NB = 3
XC = 4
XR = S // XC


def _silu(t):
    h = 0.5 * t
    return h * jnp.tanh(h) + h


def make_order(order, n):
    if isinstance(order, str):
        return order.split()
    seq = []
    if order == 3:
        seq += ['T1', 'K00', 'K01']
        for j in range(n):
            if j + 1 < n:
                seq += [f'Q{j+1}', f'K{j+1}0', f'K{j+1}1']
            seq += [f'S{j}0', f'S{j}1', f'V{j}0', f'V{j}1']
            if j == n - 1:
                seq += ['W0', 'T0', 'T2', 'T3', 'Q0']
            seq += [f'O{j}']
    elif order == 4:
        seq += ['T1', 'K00', 'K01']
        for j in range(n):
            if j + 1 < n:
                seq += [f'Q{j+1}', f'K{j+1}0', f'K{j+1}1']
            if j == n - 1:
                seq += ['W0', 'T0', 'T2', 'T3', 'Q0']
            seq += [f'S{j}0', f'S{j}1', f'V{j}0', f'V{j}1']
            seq += [f'O{j}']
    elif order == 5:
        seq += ['T1', 'K00', 'K01']
        for j in range(n):
            if j + 1 < n:
                seq += [f'Q{j+1}', f'K{j+1}0', f'K{j+1}1']
            seq += [f'S{j}0', f'S{j}1', f'V{j}0', f'V{j}1']
            seq += [f'O{j}']
        seq += ['W0', 'T0', 'T2', 'T3', 'Q0']
    return seq


def build(TM=1024, order=5, wtop=True):
    n = S // TM
    c = (DH ** -0.5) * LOG2E

    def kernel(x_hbm, kT_hbm, vT_hbm, wq_hbm, wo_hbm, wr_ref, wg_hbm, wu_hbm, wd_hbm, o_hbm,
               x_ref, xT_ref, xnT_ref, acc_ref, xs_ref, upd_ref, idx_ref, r_ref,
               wq_b, wo_b, k_b, v_b, wqT_ref, woT_ref, k_ref, q0_ref, wg_ref, wu_ref, wd_ref,
               x_sem, w_sem, m_sem, o_sem):

        def x_copy(cc):
            return pltpu.make_async_copy(x_hbm.at[pl.ds(cc * XR, XR), :], x_ref.at[pl.ds(cc * XR, XR), :], x_sem.at[cc])

        def w_copies(p, slot):
            off = pl.multiple_of(p * PAIR, 128)
            return [
                pltpu.make_async_copy(wq_hbm.at[:, pl.ds(off, PAIR)], wq_b.at[slot], w_sem.at[0, slot]),
                pltpu.make_async_copy(kT_hbm.at[pl.ds(off, PAIR), pl.ds(SK - W, W)], k_b.at[slot], w_sem.at[1, slot]),
                pltpu.make_async_copy(vT_hbm.at[pl.ds(off, PAIR), pl.ds(SK - W, W)], v_b.at[slot], w_sem.at[2, slot]),
                pltpu.make_async_copy(wo_hbm.at[pl.ds(off, PAIR), :], wo_b.at[slot], w_sem.at[3, slot]),
            ]

        m_copies = [pltpu.make_async_copy(s_, d_, m_sem.at[t]) for t, (s_, d_) in
                    enumerate(((wg_hbm, wg_ref), (wu_hbm, wu_ref), (wd_hbm, wd_ref)))]

        def o_copy(cc):
            return pltpu.make_async_copy(x_ref.at[pl.ds(cc * XR, XR), :], o_hbm.at[pl.ds(cc * XR, XR), :], o_sem.at[cc])

        for cc in range(XC):
            x_copy(cc).start()
        for cp in w_copies(0, 0):
            cp.start()
        for cp in w_copies(1, 1):
            cp.start()
        acc_ref[...] = jnp.zeros_like(acc_ref)
        wrc = jnp.broadcast_to(wr_ref[...].astype(f32).reshape(1, D), (128, D)).T
        for cc in range(XC):
            x_copy(cc).wait()
            for t in range(cc * XR // 128, (cc + 1) * XR // 128):
                cols = slice(t * 128, (t + 1) * 128)
                xT = x_ref[cols, :].T
                xT_ref[:, cols] = xT
                xf = xT.astype(f32)
                m = jnp.sum(xf, axis=0, keepdims=True) * (1.0 / D)
                xc = xf - m
                v = jnp.sum(xc * xc, axis=0, keepdims=True) * (1.0 / D)
                xn = xc * lax.rsqrt(v + 1e-5)
                xnT_ref[:, cols] = xn.astype(bf16)
                r_ref[t:t + 1, :] = jnp.sum(xn * wrc, axis=0, keepdims=True)
        for cp in m_copies:
            cp.start()
        r = r_ref[...].astype(bf16).astype(f32)
        tok = lax.broadcasted_iota(jnp.int32, (S // 128, 128), 0) * 128 + lax.broadcasted_iota(jnp.int32, (S // 128, 128), 1)
        m1 = jnp.max(r)
        i1 = jnp.minimum(jnp.min(jnp.where(r == m1, tok, S)), S - 1)
        r2 = jnp.where(tok == i1, -jnp.inf, r)
        m2 = jnp.max(r2)
        i2 = jnp.minimum(jnp.min(jnp.where(r2 == m2, tok, S)), S - 1)
        idx_ref[0] = i1
        idx_ref[1] = i2
        r16 = lax.broadcasted_iota(jnp.int32, (16, 1), 0)
        rows = []
        for ii in (i1, i2):
            base = pl.multiple_of((ii // 16) * 16, 16)
            blk = x_ref[pl.ds(base, 16), :].astype(f32)
            rows.append(jnp.sum(jnp.where(r16 == ii - base, blk, 0.0), axis=0, keepdims=True))
        xs = jnp.where(r16 == 0, rows[0], jnp.where(r16 == 1, rows[1], 0.0))
        m = jnp.mean(xs, axis=-1, keepdims=True)
        xc = xs - m
        v = jnp.mean(xc * xc, axis=-1, keepdims=True)
        xs_ref[...] = (xc * lax.rsqrt(v + 1e-5)).astype(bf16)
        upd_ref[...] = jax.nn.sigmoid(jnp.where(r16 == 0, m1, m2) + jnp.zeros((16, D), f32))

        def t_q(slot):
            wqT_ref[...] = wq_b[slot].T

        def t_k(slot, h):
            k_ref[h] = k_b[slot, h * DH:(h + 1) * DH, :].T

        def qproj(j):
            cols = pl.ds(j * TM, TM)
            return (jnp.dot(wqT_ref[...], xnT_ref[:, cols], preferred_element_type=f32) * c).astype(bf16)

        def qk(qT, h):
            return jnp.dot(k_ref[h], qT[h * DH:(h + 1) * DH], preferred_element_type=f32)

        def sm(s):
            mx = jnp.max(s, axis=0, keepdims=True)
            p = jnp.exp2(s - mx)
            l = jnp.sum(p, axis=0, keepdims=True)
            return p.astype(bf16), l

        def pv(p, l, h, slot):
            o = jnp.dot(v_b[slot, h * DH:(h + 1) * DH, :], p, preferred_element_type=f32)
            return (o * (1.0 / l)).astype(bf16)

        def oproj(j, o0, o1):
            cols = pl.ds(j * TM, TM)
            o2 = jnp.concatenate([o0, o1], axis=0)
            acc_ref[:, cols] += jnp.dot(woT_ref[...], o2, preferred_element_type=f32)

        for cp in w_copies(0, 0):
            cp.wait()
        t_q(0)
        t_k(0, 0)
        t_k(0, 1)
        q0_ref[...] = qproj(0)

        def body(p, carry):
            slot = lax.rem(p, NB)
            nslot = lax.rem(p + 1, NB)
            pn = jnp.minimum(p + 1, NP - 1)

            @pl.when(p + 2 < NP)
            def _():
                for cp in w_copies(p + 2, lax.rem(p + 2, NB)):
                    cp.start()

            def wait_next():
                @pl.when(p + 1 < NP)
                def _():
                    for cp in w_copies(p + 1, nslot):
                        cp.wait()

            @pl.when(p == 2)
            def _():
                for cp in m_copies:
                    cp.wait()
                xs = xs_ref[...]
                g = jnp.dot(xs, wg_ref[...], preferred_element_type=f32)
                u = jnp.dot(xs, wu_ref[...], preferred_element_type=f32)
                hdn = (_silu(g) * u).astype(bf16)
                upd_ref[...] = upd_ref[...] * jnp.dot(hdn, wd_ref[...], preferred_element_type=f32)

            if wtop:
                wait_next()
            ns = jnp.where(p + 1 < NP, nslot, slot)
            st = {('q', 0): q0_ref[...]}
            for tok in make_order(order, n):
                kind, j = tok[0], int(tok[1])
                h = int(tok[2]) if len(tok) > 2 else None
                if kind == 'Q':
                    if j == 0:
                        q0_ref[...] = qproj(0)
                    else:
                        st['q', j] = qproj(j)
                elif kind == 'K':
                    st['s', j, h] = qk(st['q', j], h)
                elif kind == 'S':
                    st['p', j, h] = sm(st.pop(('s', j, h)))
                elif kind == 'V':
                    st['o', j, h] = pv(*st.pop(('p', j, h)), h, slot)
                elif kind == 'O':
                    oproj(j, st.pop(('o', j, 0)), st.pop(('o', j, 1)))
                elif kind == 'W':
                    if not wtop:
                        wait_next()
                elif kind == 'T':
                    if j == 0:
                        t_q(ns)
                    elif j == 1:
                        woT_ref[...] = wo_b[slot].T
                    else:
                        t_k(ns, j - 2)
            return carry

        lax.fori_loop(0, NP, body, 0)

        upd = upd_ref[...]
        u1 = jnp.broadcast_to(upd[0:1, :], (128, D)).T
        u2 = jnp.broadcast_to(upd[1:2, :], (128, D)).T
        lane = lax.broadcasted_iota(jnp.int32, (D, 128), 1)
        i1 = idx_ref[0]
        i2 = idx_ref[1]
        for cc in range(XC):
            for t in range(cc * XR // 128, (cc + 1) * XR // 128):
                cols = slice(t * 128, (t + 1) * 128)
                tt = xnT_ref[:, cols].astype(f32) + jnp.where(lane == i1 - t * 128, u1, jnp.where(lane == i2 - t * 128, u2, 0.0))
                res = xT_ref[:, cols].astype(f32) + acc_ref[:, cols] * _silu(tt)
                x_ref[cols, :] = res.astype(bf16).T
            o_copy(cc).start()
        for cc in range(XC):
            o_copy(cc).wait()

    def f(A_x, A_k_cache, A_v_cache, A_wq, A_wo, B_x, B_w_r, B_w_gate, B_w_up, B_w_down):
        x = A_x.reshape(S, D)
        kT = jnp.swapaxes(A_k_cache, 2, 3).reshape(H * DH, SK)
        vT = jnp.swapaxes(A_v_cache, 2, 3).reshape(H * DH, SK)
        hbm = pl.BlockSpec(memory_space=pl.ANY)
        out = pl.pallas_call(
            kernel,
            in_specs=[hbm, hbm, hbm, hbm, hbm, pl.BlockSpec(memory_space=pltpu.VMEM), hbm, hbm, hbm],
            out_specs=hbm,
            out_shape=jax.ShapeDtypeStruct((S, D), bf16),
            scratch_shapes=[
                pltpu.VMEM((S, D), bf16),
                pltpu.VMEM((D, S), bf16),
                pltpu.VMEM((D, S), bf16),
                pltpu.VMEM((D, S), f32),
                pltpu.VMEM((16, D), bf16),
                pltpu.VMEM((16, D), f32),
                pltpu.SMEM((2,), jnp.int32),
                pltpu.VMEM((S // 128, 128), f32),
                pltpu.VMEM((NB, D, PAIR), bf16),
                pltpu.VMEM((NB, PAIR, D), bf16),
                pltpu.VMEM((NB, PAIR, W), bf16),
                pltpu.VMEM((NB, PAIR, W), bf16),
                pltpu.VMEM((PAIR, D), bf16),
                pltpu.VMEM((D, PAIR), bf16),
                pltpu.VMEM((2, W, DH), bf16),
                pltpu.VMEM((PAIR, TM), bf16),
                pltpu.VMEM((D, F), bf16),
                pltpu.VMEM((D, F), bf16),
                pltpu.VMEM((F, D), bf16),
                pltpu.SemaphoreType.DMA((XC,)),
                pltpu.SemaphoreType.DMA((4, NB)),
                pltpu.SemaphoreType.DMA((3,)),
                pltpu.SemaphoreType.DMA((XC,)),
            ],
            compiler_params=pltpu.CompilerParams(vmem_limit_bytes=100 * 1024 * 1024),
        )(x, kT, vT, A_wq, A_wo, B_w_r, B_w_gate, B_w_up, B_w_down)
        return out.reshape(1, S, D)
    return f

pallas_recurrent_scan__sliding_block_cached__moe_arch_mod__prompt_kernel = jax.jit(build())
```

```python
import functools
import jax
import jax.numpy as jnp
import numpy as np
from jax import lax
from jax.experimental import pallas as pl
from jax.experimental.pallas import tpu as pltpu

S, D, H, DH, SK, F = 2048, 640, 32, 192, 2048, 1536
W = 512
PAIR = 2 * DH
NP = H // 2
LOG2E = 1.4426950408889634
f32 = jnp.float32
bf16 = jnp.bfloat16
NB = 2
XC = 4
XR = S // XC


def _silu(t):
    h = 0.5 * t
    return h * jnp.tanh(h) + h


def _tree(xs):
    xs = list(xs)
    while len(xs) > 1:
        xs = [xs[i] + xs[i + 1] if i + 1 < len(xs) else xs[i] for i in range(0, len(xs), 2)]
    return xs[0]


def make_order(order, n):
    if isinstance(order, str):
        return order.split()
    seq = []
    if order == 3:
        seq += ['T1', 'K00', 'K01']
        for j in range(n):
            if j + 1 < n:
                seq += [f'Q{j+1}', f'K{j+1}0', f'K{j+1}1']
            seq += [f'S{j}0', f'S{j}1', f'V{j}0', f'V{j}1']
            if j == n - 1:
                seq += ['W0', 'T0', 'T2', 'T3', 'Q0']
            seq += [f'O{j}']
    elif order == 4:
        seq += ['T1', 'K00', 'K01']
        for j in range(n):
            if j + 1 < n:
                seq += [f'Q{j+1}', f'K{j+1}0', f'K{j+1}1']
            if j == n - 1:
                seq += ['W0', 'T0', 'T2', 'T3', 'Q0']
            seq += [f'S{j}0', f'S{j}1', f'V{j}0', f'V{j}1']
            seq += [f'O{j}']
    elif order == 5:
        seq += ['T1', 'K00', 'K01']
        for j in range(n):
            if j + 1 < n:
                seq += [f'Q{j+1}', f'K{j+1}0', f'K{j+1}1']
            seq += [f'S{j}0', f'S{j}1', f'V{j}0', f'V{j}1']
            seq += [f'O{j}']
        seq += ['W0', 'T0', 'T2', 'T3', 'Q0']
    return seq


def build(OC=16, gate_pos=0, carry=False, CH=(2048,), order='T1 Q0 K00 K01 S00 S01 V00 V01 T0 T2 T3 O0', wtop=True, kpad=False, ln2=True, rmxu=False, t2late=True):
    n = len(CH)
    OFF = [sum(CH[:j]) for j in range(n)]
    assert sum(CH) == S
    c = (DH ** -0.5) * LOG2E

    def kernel(x_hbm, kT_hbm, vT_hbm, wq_hbm, wo_hbm, wr_ref, wg_hbm, wu_hbm, wd_hbm, o_hbm,
               x_ref, xn_ref, xnT_ref, acc_ref, xs_ref, upd_ref, idx_ref, r_ref,
               wq_b, wo_b, k_b, v_b, wqT_ref, woT_ref, k_ref, q0_ref, wg_ref, wu_ref, wd_ref,
               x_sem, w_sem, m_sem, o_sem):

        def x_copy(cc):
            return pltpu.make_async_copy(x_hbm.at[pl.ds(cc * XR, XR), :], x_ref.at[pl.ds(cc * XR, XR), :], x_sem.at[cc])

        def a_copies(p, slot):
            off = pl.multiple_of(p * PAIR, 128)
            return [
                pltpu.make_async_copy(wq_hbm.at[:, pl.ds(off, PAIR)], wq_b.at[slot], w_sem.at[0, slot]),
                pltpu.make_async_copy(kT_hbm.at[pl.ds(off, PAIR), pl.ds(SK - W, W)], k_b.at[slot], w_sem.at[1, slot]),
            ]

        def b_copies(p, slot):
            off = pl.multiple_of(p * PAIR, 128)
            return [
                pltpu.make_async_copy(vT_hbm.at[pl.ds(off, PAIR), pl.ds(SK - W, W)], v_b.at[slot], w_sem.at[2, slot]),
                pltpu.make_async_copy(wo_hbm.at[pl.ds(off, PAIR), :], wo_b.at[slot], w_sem.at[3, slot]),
            ]

        m_copies = [pltpu.make_async_copy(s_, d_, m_sem.at[t]) for t, (s_, d_) in
                    enumerate(((wg_hbm, wg_ref), (wu_hbm, wu_ref), (wd_hbm, wd_ref)))]

        def o_copy(cc):
            n_ = S // OC
            return pltpu.make_async_copy(x_ref.at[pl.ds(cc * n_, n_), :], o_hbm.at[pl.ds(cc * n_, n_), :], o_sem.at[cc])

        for cc in range(XC):
            x_copy(cc).start()
        for cp in a_copies(0, 0) + b_copies(0, 0) + a_copies(1, 1):
            cp.start()
        acc_ref[...] = jnp.zeros_like(acc_ref)
        wr = wr_ref[...].astype(f32).reshape(1, D)
        for cc in range(XC):
            x_copy(cc).wait()
            for t in range(cc * XR // 128, (cc + 1) * XR // 128):
                rows = slice(t * 128, (t + 1) * 128)
                xf = x_ref[rows, :].astype(f32)
                m = jnp.sum(_tree([xf[:, k * 128:(k + 1) * 128] for k in range(5)]), axis=1, keepdims=True) * (1.0 / D)
                xc = xf - m
                sq = xc * xc
                v = jnp.sum(_tree([sq[:, k * 128:(k + 1) * 128] for k in range(5)]), axis=1, keepdims=True) * (1.0 / D)
                xn_ref[rows, :] = (xc * lax.rsqrt(v + 1e-5)).astype(bf16)
                xnT_ref[:, rows] = xn_ref[rows, :].T
        wr16 = jnp.broadcast_to(wr_ref[...].reshape(1, D), (16, D))
        rr = jnp.dot(wr16, xnT_ref[...], preferred_element_type=f32)
        for t in range(S // 128):
            r_ref[t:t + 1, :] = rr[0:1, t * 128:(t + 1) * 128]
        for cp in m_copies:
            cp.start()
        def top2():
            r = r_ref[...].astype(bf16).astype(f32)
            tok = lax.broadcasted_iota(jnp.int32, (S // 128, 128), 0) * 128 + lax.broadcasted_iota(jnp.int32, (S // 128, 128), 1)
            m1 = jnp.max(r)
            i1 = jnp.minimum(jnp.min(jnp.where(r == m1, tok, S)), S - 1)
            r2 = jnp.where(tok == i1, -jnp.inf, r)
            m2 = jnp.max(r2)
            i2 = jnp.minimum(jnp.min(jnp.where(r2 == m2, tok, S)), S - 1)
            idx_ref[0] = i1
            idx_ref[1] = i2
            r16 = lax.broadcasted_iota(jnp.int32, (16, 1), 0)
            rows = []
            for ii in (i1, i2):
                base = pl.multiple_of((ii // 16) * 16, 16)
                blk = x_ref[pl.ds(base, 16), :].astype(f32)
                rows.append(jnp.sum(jnp.where(r16 == ii - base, blk, 0.0), axis=0, keepdims=True))
            xs = jnp.where(r16 == 0, rows[0], jnp.where(r16 == 1, rows[1], 0.0))
            m = jnp.mean(xs, axis=-1, keepdims=True)
            xc = xs - m
            v = jnp.mean(xc * xc, axis=-1, keepdims=True)
            xs_ref[...] = (xc * lax.rsqrt(v + 1e-5)).astype(bf16)
            upd_ref[...] = jax.nn.sigmoid(jnp.where(r16 == 0, m1, m2) + jnp.zeros((16, D), f32))

        if not t2late:
            top2()

        def t_q(slot):
            wqT_ref[...] = wq_b[slot].T

        def t_k(slot, h):
            if kpad:
                k2 = k_b[slot, 128 * h:128 * h + 256, :].T
                lane = lax.broadcasted_iota(jnp.int32, (W, 256), 1)
                k_ref[h] = jnp.where((lane < DH) if h == 0 else (lane >= 64), k2, jnp.zeros((), bf16))
            else:
                k_ref[h] = k_b[slot, h * DH:(h + 1) * DH, :].T

        def qproj(j):
            cols = pl.ds(OFF[j], CH[j])
            return (jnp.dot(wqT_ref[...], xnT_ref[:, cols], preferred_element_type=f32) * c).astype(bf16)

        def qk(qT, h):
            qs = qT[128 * h:128 * h + 256] if kpad else qT[h * DH:(h + 1) * DH]
            return jnp.dot(k_ref[h], qs, preferred_element_type=f32)

        def sm(s):
            mx = jnp.max(s, axis=0, keepdims=True)
            p = jnp.exp2(s - mx)
            l = jnp.sum(p, axis=0, keepdims=True)
            return p.astype(bf16), l

        def pv(p, l, h, slot):
            o = jnp.dot(v_b[slot, h * DH:(h + 1) * DH, :], p, preferred_element_type=f32)
            return (o * (1.0 / l)).astype(bf16)

        def oproj(j, o0, o1):
            cols = pl.ds(OFF[j], CH[j])
            o2 = jnp.concatenate([o0, o1], axis=0)
            acc_ref[:, cols] += jnp.dot(woT_ref[...], o2, preferred_element_type=f32)

        for cp in a_copies(0, 0):
            cp.wait()
        t_q(0)
        t_k(0, 0)
        t_k(0, 1)
        if carry:
            q0_ref[...] = qproj(0)
        if t2late:
            top2()

        def body(p, carry_):
            slot = lax.rem(p, NB)
            nslot = lax.rem(p + 1, NB)
            pn = jnp.minimum(p + 1, NP - 1)

            for cp in b_copies(p, slot):
                cp.wait()

            @pl.when(p + 1 < NP)
            def _():
                for cp in a_copies(p + 1, nslot):
                    cp.wait()
                for cp in b_copies(p + 1, nslot):
                    cp.start()

            @pl.when(p + 2 < NP)
            def _():
                for cp in a_copies(p + 2, slot):
                    cp.start()

            @pl.when(p == 2)
            def _():
                for cp in m_copies:
                    cp.wait()
                xs = xs_ref[...]
                g = jnp.dot(xs, wg_ref[...], preferred_element_type=f32)
                u = jnp.dot(xs, wu_ref[...], preferred_element_type=f32)
                hdn = (_silu(g) * u).astype(bf16)
                upd = (upd_ref[...] * jnp.dot(hdn, wd_ref[...], preferred_element_type=f32).astype(bf16).astype(f32)).astype(bf16)
                upd_ref[...] = xs.astype(f32) + upd.astype(f32)

            ns = jnp.where(p + 1 < NP, nslot, slot)
            def gate():
                rows = pl.ds(pl.multiple_of(p * 128, 128), 128)
                g_ref[rows, :] = _silu(xn_ref[rows, :].astype(f32)).astype(bf16)

            st = {('q', 0): q0_ref[...]} if carry else {}
            for tok in make_order(order, n):
                kind, j = tok[0], int(tok[1])
                h = int(tok[2]) if len(tok) > 2 else None
                if kind == 'Q':
                    if j == 0 and carry:
                        q0_ref[...] = qproj(0)
                    else:
                        st['q', j] = qproj(j)
                elif kind == 'K':
                    st['s', j, h] = qk(st['q', j], h)
                elif kind == 'S':
                    st['p', j, h] = sm(st.pop(('s', j, h)))
                elif kind == 'V':
                    st['o', j, h] = pv(*st.pop(('p', j, h)), h, slot)
                elif kind == 'O':
                    oproj(j, st.pop(('o', j, 0)), st.pop(('o', j, 1)))
                elif kind == 'G':
                    gate()
                elif kind == 'T':
                    if j == 0:
                        t_q(ns)
                    elif j == 1:
                        woT_ref[...] = wo_b[slot].T
                    else:
                        t_k(ns, j - 2)
            return carry_

        lax.fori_loop(0, NP, body, 0)

        r16 = lax.broadcasted_iota(jnp.int32, (16, 1), 0)
        for kk in range(2):
            ii = idx_ref[kk]
            blk = pl.ds(pl.multiple_of((ii // 16) * 16, 16), 16)
            xn_ref[blk, :] = jnp.where(r16 == ii % 16, upd_ref[kk:kk + 1, :], xn_ref[blk, :].astype(f32)).astype(bf16)
        OR = S // OC
        for cc in range(OC):
            for t in range(cc * OR // 128, (cc + 1) * OR // 128):
                rows = slice(t * 128, (t + 1) * 128)
                s = acc_ref[:, rows].astype(bf16).T.astype(f32)
                x_ref[rows, :] = (x_ref[rows, :].astype(f32) + s * _silu(xn_ref[rows, :].astype(f32))).astype(bf16)
            o_copy(cc).start()
        for cc in range(OC):
            o_copy(cc).wait()

    def f(A_x, A_k_cache, A_v_cache, A_wq, A_wo, B_x, B_w_r, B_w_gate, B_w_up, B_w_down):
        x = A_x.reshape(S, D)
        kT = jnp.swapaxes(A_k_cache, 2, 3).reshape(H * DH, SK)
        vT = jnp.swapaxes(A_v_cache, 2, 3).reshape(H * DH, SK)
        hbm = pl.BlockSpec(memory_space=pl.ANY)
        out = pl.pallas_call(
            kernel,
            in_specs=[hbm, hbm, hbm, hbm, hbm, pl.BlockSpec(memory_space=pltpu.VMEM), hbm, hbm, hbm],
            out_specs=hbm,
            out_shape=jax.ShapeDtypeStruct((S, D), bf16),
            scratch_shapes=[
                pltpu.VMEM((S, D), bf16),
                pltpu.VMEM((S, D), bf16),
                pltpu.VMEM((D, S), bf16),
                pltpu.VMEM((D, S), f32),
                pltpu.VMEM((16, D), bf16),
                pltpu.VMEM((16, D), f32),
                pltpu.SMEM((2,), jnp.int32),
                pltpu.VMEM((S // 128, 128), f32),
                pltpu.VMEM((NB, D, PAIR), bf16),
                pltpu.VMEM((NB, PAIR, D), bf16),
                pltpu.VMEM((NB, PAIR, W), bf16),
                pltpu.VMEM((NB, PAIR, W), bf16),
                pltpu.VMEM((PAIR, D), bf16),
                pltpu.VMEM((D, PAIR), bf16),
                pltpu.VMEM((2, W, 256 if kpad else DH), bf16),
                pltpu.VMEM((PAIR, CH[0]), bf16),
                pltpu.VMEM((D, F), bf16),
                pltpu.VMEM((D, F), bf16),
                pltpu.VMEM((F, D), bf16),
                pltpu.SemaphoreType.DMA((XC,)),
                pltpu.SemaphoreType.DMA((4, NB)),
                pltpu.SemaphoreType.DMA((3,)),
                pltpu.SemaphoreType.DMA((OC,)),
            ],
            compiler_params=pltpu.CompilerParams(vmem_limit_bytes=100 * 1024 * 1024),
        )(x, kT, vT, A_wq, A_wo, B_w_r, B_w_gate, B_w_up, B_w_down)
        return out.reshape(1, S, D)
    return f

pallas_recurrent_scan__sliding_block_cached__moe_arch_mod__prompt_kernel = jax.jit(build())
```

```python
import jax
import jax.numpy as jnp
from jax import lax
from jax.experimental import pallas as pl
from jax.experimental.pallas import tpu as pltpu

S, D, H, DH, SK, F = 2048, 640, 32, 192, 2048, 1536
W = min(4096, max(256, SK // 4))
PAIR = 2 * DH
NP = H // 2
NB = 2
XC = 8
OC = 16
LOG2E = 1.4426950408889634
QSCALE = (DH ** -0.5) * LOG2E
EPS = 1e-5
f32 = jnp.float32
bf16 = jnp.bfloat16


def _silu(t):
    h = 0.5 * t
    return h * jnp.tanh(h) + h


def _lane_sum(a):
    parts = [a[:, k * 128:(k + 1) * 128] for k in range(a.shape[1] // 128)]
    while len(parts) > 1:
        parts = [parts[i] + parts[i + 1] if i + 1 < len(parts) else parts[i]
                 for i in range(0, len(parts), 2)]
    return jnp.sum(parts[0], axis=1, keepdims=True)


def _layernorm(xf):
    m = _lane_sum(xf) * (1.0 / D)
    xc = xf - m
    v = _lane_sum(xc * xc) * (1.0 / D)
    return xc * lax.rsqrt(v + EPS)


def _kernel(x_hbm, kT_hbm, vT_hbm, wq_hbm, wo_hbm, wr_ref, wg_hbm, wu_hbm, wd_hbm, o_hbm,
            x_ref, xn_ref, xnT_ref, acc_ref, xs_ref, upd_ref, idx_ref, r_ref,
            wq_b, wo_b, k_b, v_b, wqT_ref, woT_ref, k_ref, wg_ref, wu_ref, wd_ref,
            x_sem, w_sem, m_sem, o_sem):

    def x_copy(c):
        n = S // XC
        return pltpu.make_async_copy(x_hbm.at[pl.ds(c * n, n), :], x_ref.at[pl.ds(c * n, n), :], x_sem.at[c])

    def o_copy(c):
        n = S // OC
        return pltpu.make_async_copy(x_ref.at[pl.ds(c * n, n), :], o_hbm.at[pl.ds(c * n, n), :], o_sem.at[c])

    def a_copies(p, slot):
        off = pl.multiple_of(p * PAIR, 128)
        return [
            pltpu.make_async_copy(wq_hbm.at[:, pl.ds(off, PAIR)], wq_b.at[slot], w_sem.at[0, slot]),
            pltpu.make_async_copy(kT_hbm.at[pl.ds(off, PAIR), pl.ds(SK - W, W)], k_b.at[slot], w_sem.at[1, slot]),
        ]

    def b_copies(p, slot):
        off = pl.multiple_of(p * PAIR, 128)
        return [
            pltpu.make_async_copy(vT_hbm.at[pl.ds(off, PAIR), pl.ds(SK - W, W)], v_b.at[slot], w_sem.at[2, slot]),
            pltpu.make_async_copy(wo_hbm.at[pl.ds(off, PAIR), :], wo_b.at[slot], w_sem.at[3, slot]),
        ]

    m_copies = [pltpu.make_async_copy(src, dst, m_sem.at[t]) for t, (src, dst) in
                enumerate(((wg_hbm, wg_ref), (wu_hbm, wu_ref), (wd_hbm, wd_ref)))]

    for cp in [x_copy(c) for c in range(XC)] + a_copies(0, 0) + b_copies(0, 0) + a_copies(1, 1):
        cp.start()
    acc_ref[...] = jnp.zeros_like(acc_ref)
    for c in range(XC):
        x_copy(c).wait()
        for t in range(c * S // XC // 128, (c + 1) * S // XC // 128):
            rows = slice(t * 128, (t + 1) * 128)
            xn_ref[rows, :] = _layernorm(x_ref[rows, :].astype(f32)).astype(bf16)
            xnT_ref[:, rows] = xn_ref[rows, :].T
    wr16 = jnp.broadcast_to(wr_ref[...].reshape(1, D), (16, D))
    rr = jnp.dot(wr16, xnT_ref[...], preferred_element_type=f32)
    for t in range(S // 128):
        r_ref[t:t + 1, :] = rr[0:1, t * 128:(t + 1) * 128]
    for cp in m_copies:
        cp.start()

    def t_q(slot):
        wqT_ref[...] = wq_b[slot].T

    def t_k(slot, h):
        k_ref[h] = k_b[slot, h * DH:(h + 1) * DH, :].T

    for cp in a_copies(0, 0):
        cp.wait()
    t_q(0)
    t_k(0, 0)
    t_k(0, 1)

    r = r_ref[...].astype(bf16).astype(f32)
    tok = (lax.broadcasted_iota(jnp.int32, (S // 128, 128), 0) * 128
           + lax.broadcasted_iota(jnp.int32, (S // 128, 128), 1))
    m1 = jnp.max(r)
    i1 = jnp.minimum(jnp.min(jnp.where(r == m1, tok, S)), S - 1)
    r2 = jnp.where(tok == i1, -jnp.inf, r)
    m2 = jnp.max(r2)
    i2 = jnp.minimum(jnp.min(jnp.where(r2 == m2, tok, S)), S - 1)
    idx_ref[0] = i1
    idx_ref[1] = i2
    r16 = lax.broadcasted_iota(jnp.int32, (16, 1), 0)
    sel = []
    for ii in (i1, i2):
        base = pl.multiple_of((ii // 16) * 16, 16)
        blk = x_ref[pl.ds(base, 16), :].astype(f32)
        sel.append(jnp.sum(jnp.where(r16 == ii - base, blk, 0.0), axis=0, keepdims=True))
    xs = jnp.where(r16 == 0, sel[0], jnp.where(r16 == 1, sel[1], 0.0))
    xs_ref[...] = _layernorm(xs).astype(bf16)
    upd_ref[...] = jax.nn.sigmoid(jnp.where(r16 == 0, m1, m2) + jnp.zeros((16, D), f32))

    def qk(qT, h):
        return jnp.dot(k_ref[h], qT[h * DH:(h + 1) * DH], preferred_element_type=f32)

    def softmax(s):
        mx = jnp.max(s, axis=0, keepdims=True)
        p = jnp.exp2(s - mx)
        return p.astype(bf16), jnp.sum(p, axis=0, keepdims=True)

    def pv(p, l, h, slot):
        o = jnp.dot(v_b[slot, h * DH:(h + 1) * DH, :], p, preferred_element_type=f32)
        return (o * (1.0 / l)).astype(bf16)

    def body(p, carry):
        slot = lax.rem(p, NB)
        nslot = lax.rem(p + 1, NB)
        for cp in b_copies(p, slot):
            cp.wait()

        @pl.when(p + 1 < NP)
        def _():
            for cp in a_copies(p + 1, nslot):
                cp.wait()
            for cp in b_copies(p + 1, nslot):
                cp.start()

        @pl.when(p + 2 < NP)
        def _():
            for cp in a_copies(p + 2, slot):
                cp.start()

        @pl.when(p == 2)
        def _():
            for cp in m_copies:
                cp.wait()
            xsel = xs_ref[...]
            g = jnp.dot(xsel, wg_ref[...], preferred_element_type=f32)
            u = jnp.dot(xsel, wu_ref[...], preferred_element_type=f32)
            hdn = (_silu(g) * u).astype(bf16)
            y = jnp.dot(hdn, wd_ref[...], preferred_element_type=f32).astype(bf16).astype(f32)
            upd = (upd_ref[...] * y).astype(bf16)
            upd_ref[...] = xsel.astype(f32) + upd.astype(f32)

        ns = jnp.where(p + 1 < NP, nslot, slot)
        woT_ref[...] = wo_b[slot].T
        qT = (jnp.dot(wqT_ref[...], xnT_ref[...], preferred_element_type=f32) * QSCALE).astype(bf16)
        s0 = qk(qT, 0)
        s1 = qk(qT, 1)
        p0, l0 = softmax(s0)
        p1, l1 = softmax(s1)
        o0 = pv(p0, l0, 0, slot)
        o1 = pv(p1, l1, 1, slot)
        t_q(ns)
        t_k(ns, 0)
        t_k(ns, 1)
        o2 = jnp.concatenate([o0, o1], axis=0)
        acc_ref[...] += jnp.dot(woT_ref[...], o2, preferred_element_type=f32)
        return carry

    lax.fori_loop(0, NP, body, 0)

    for kk in range(2):
        ii = idx_ref[kk]
        blk = pl.ds(pl.multiple_of((ii // 16) * 16, 16), 16)
        xn_ref[blk, :] = jnp.where(r16 == ii % 16, upd_ref[kk:kk + 1, :],
                                   xn_ref[blk, :].astype(f32)).astype(bf16)
    for c in range(OC):
        for t in range(c * S // OC // 128, (c + 1) * S // OC // 128):
            rows = slice(t * 128, (t + 1) * 128)
            s = acc_ref[:, rows].astype(bf16).T.astype(f32)
            gate = _silu(xn_ref[rows, :].astype(f32))
            x_ref[rows, :] = (x_ref[rows, :].astype(f32) + s * gate).astype(bf16)
        o_copy(c).start()
    for c in range(OC):
        o_copy(c).wait()


@jax.jit
def pallas_recurrent_scan__sliding_block_cached__moe_arch_mod__prompt_kernel(
    A_x: jax.Array,
    A_k_cache: jax.Array,
    A_v_cache: jax.Array,
    A_wq: jax.Array,
    A_wo: jax.Array,
    B_x: jax.Array,
    B_w_r: jax.Array,
    B_w_gate: jax.Array,
    B_w_up: jax.Array,
    B_w_down: jax.Array,
):
    del B_x
    x = A_x.reshape(S, D)
    kT = jnp.swapaxes(A_k_cache, 2, 3).reshape(H * DH, SK)
    vT = jnp.swapaxes(A_v_cache, 2, 3).reshape(H * DH, SK)
    hbm = pl.BlockSpec(memory_space=pl.ANY)
    out = pl.pallas_call(
        _kernel,
        in_specs=[hbm, hbm, hbm, hbm, hbm, pl.BlockSpec(memory_space=pltpu.VMEM), hbm, hbm, hbm],
        out_specs=hbm,
        out_shape=jax.ShapeDtypeStruct((S, D), bf16),
        scratch_shapes=[
            pltpu.VMEM((S, D), bf16),
            pltpu.VMEM((S, D), bf16),
            pltpu.VMEM((D, S), bf16),
            pltpu.VMEM((D, S), f32),
            pltpu.VMEM((16, D), bf16),
            pltpu.VMEM((16, D), f32),
            pltpu.SMEM((2,), jnp.int32),
            pltpu.VMEM((S // 128, 128), f32),
            pltpu.VMEM((NB, D, PAIR), bf16),
            pltpu.VMEM((NB, PAIR, D), bf16),
            pltpu.VMEM((NB, PAIR, W), bf16),
            pltpu.VMEM((NB, PAIR, W), bf16),
            pltpu.VMEM((PAIR, D), bf16),
            pltpu.VMEM((D, PAIR), bf16),
            pltpu.VMEM((2, W, DH), bf16),
            pltpu.VMEM((D, F), bf16),
            pltpu.VMEM((D, F), bf16),
            pltpu.VMEM((F, D), bf16),
            pltpu.SemaphoreType.DMA((XC,)),
            pltpu.SemaphoreType.DMA((4, NB)),
            pltpu.SemaphoreType.DMA((3,)),
            pltpu.SemaphoreType.DMA((OC,)),
        ],
        compiler_params=pltpu.CompilerParams(vmem_limit_bytes=100 * 1024 * 1024),
    )(x, kT, vT, A_wq, A_wo, B_w_r, B_w_gate, B_w_up, B_w_down)
    return out.reshape(1, S, D)
```
